```python
import jax
import jax.numpy as jnp

def _softmax(x, axis=-1):
    return jax.nn.softmax(x, axis=axis)
def _gelu(x):
    return jax.nn.gelu(x, approximate=True)
def _silu(x):
    return jax.nn.silu(x)
def _sigmoid(x):
    return jax.nn.sigmoid(x)
def _layernorm(x, axis=-1, eps=1e-5):
    m = jnp.mean(x, axis=axis, keepdims=True)
    v = jnp.var(x, axis=axis, keepdims=True)
    return (x - m) / jnp.sqrt(v + eps)
def _scatter_add(tgt, idx, src, axis=0):
    return tgt.at[idx].add(src)
def _segment_sum(src, seg, n):
    return jax.ops.segment_sum(src, seg, n)
class _Rng:
    def __init__(self, key):
        self._k = key
    def _next(self):
        self._k, sub = jax.random.split(self._k)
        return sub
    def normal(self, shape):
        return jax.random.normal(self._next(), shape, dtype=jnp.bfloat16)
    def randint(self, lo, hi, shape):
        return jax.random.randint(self._next(), shape, lo, hi, dtype=jnp.int32)
    def uniform(self, shape, lo=0.0, hi=1.0):
        return jax.random.uniform(self._next(), shape, jnp.bfloat16, lo, hi)
    def permutation(self, n):
        return jax.random.permutation(self._next(), n)


kernel_name = 'recurrent_scan__compressed_kv_cla__dense_activation_gelu__decode'

def setup_inputs():
    _rng = _Rng(jax.random.key(int.from_bytes(__import__("os").urandom(4), "little")))
    _w = (lambda a: (lambda t: t.astype(jnp.bfloat16) if jnp.issubdtype(t.dtype, jnp.floating) else t)(jnp.asarray(a)))
    def _A_setup():
        B, H, Sq, Sk, D, M = 2, 32, 1, 16384, 128, 512
        Dc = 4 * D
        return {
            "x": _w((lambda *s: _rng.normal(s) * 0.05)(B, Sq, M)),
            "c_kv": _w((lambda *s: _rng.normal(s) * 0.05)(B, Sk, Dc)),
            "w_q": _w((lambda *s: _rng.normal(s) * 0.05)(M, H, D) * (M ** -0.5)),
            "w_uk": _w((lambda *s: _rng.normal(s) * 0.05)(Dc, H, D) * (Dc ** -0.5)),
            "w_uv": _w((lambda *s: _rng.normal(s) * 0.05)(Dc, H, D) * (Dc ** -0.5)),
            "w_o": _w((lambda *s: _rng.normal(s) * 0.05)(H, D, M) * ((H * D) ** -0.5)),
        }
    _A_in = _A_setup()

    def _B_setup():
        B, S, D, F = 2, 1, 512, 1792
        return {
            "x": _w((lambda *s: _rng.normal(s) * 0.05)(B, S, D)),
            "w1": _w((lambda *s: _rng.normal(s) * 0.05)(D, F) * (D ** -0.5)),
            "b1": _w((lambda *s: _rng.normal(s) * 0.05)(F) * 0.01),
            "w2": _w((lambda *s: _rng.normal(s) * 0.05)(F, D) * (F ** -0.5)),
            "b2": _w((lambda *s: _rng.normal(s) * 0.05)(D) * 0.01),
        }
    _B_in = _B_setup()

    return {
        "A_x": _A_in["x"],
        "A_c_kv": _A_in["c_kv"],
        "A_w_q": _A_in["w_q"],
        "A_w_uk": _A_in["w_uk"],
        "A_w_uv": _A_in["w_uv"],
        "A_w_o": _A_in["w_o"],
        "B_x": _B_in["x"],
        "B_w1": _B_in["w1"],
        "B_b1": _B_in["b1"],
        "B_w2": _B_in["w2"],
        "B_b2": _B_in["b2"],
    }

def reference(A_x, A_c_kv, A_w_q, A_w_uk, A_w_uv, A_w_o, B_x, B_w1, B_b1, B_w2, B_b2):
    def _A_ref(x, c_kv, w_q, w_uk, w_uv, w_o):
        B, Sq, M = x.shape[0], x.shape[1], x.shape[2]
        Sk = c_kv.shape[1]
        H, D = w_q.shape[1], w_q.shape[2]
        q = jnp.einsum("bqm,mhd->bhqd", x, w_q)
        k = jnp.einsum("bkc,chd->bhkd", c_kv, w_uk)
        v = jnp.einsum("bkc,chd->bhkd", c_kv, w_uv)
        scores = jnp.einsum("bhqd,bhkd->bhqk", q, k) * (D ** -0.5)
        off = Sk - Sq
        qi = jnp.arange(Sq)[:, None]
        kj = jnp.arange(Sk)[None, :]
        cmask = kj <= (qi + off)
        scores = jnp.where(cmask[None, None], scores, -1e9)
        p = _softmax(scores, axis=-1)
        ctx = jnp.einsum("bhqk,bhkd->bhqd", p, v)
        return jnp.einsum("bhqd,hdm->bqm", ctx, w_o)

    def _B_ref(x, w1, b1, w2, b2):
        h = jnp.einsum("bsd,df->bsf", x, w1) + b1
        h = _gelu(h)
        return jnp.einsum("bsf,fd->bsd", h, w2) + b2

    x = A_x
    xn = _layernorm(x, axis=-1)
    s = _A_ref(xn, A_c_kv, A_w_q, A_w_uk, A_w_uv, A_w_o)
    g = _silu(_B_ref(xn, B_w1, B_b1, B_w2, B_b2))
    return x + s * g
```

```python
import contextlib
import jax
import jax.numpy as jnp
from jax import lax
import jax.experimental.pallas as pl
import jax.experimental.pallas.tpu as pltpu

F32 = jnp.float32
BF16 = jnp.bfloat16
I32 = jnp.int32

B, H, SK, D, M, DC, F = 2, 32, 16384, 128, 512, 512, 1792
LOG2E = 1.4426950408889634
NT = (((1,), (1,)), ((), ()))


def make_kernel(lead=4, head_p1=24, cstreams=32, name=None, last_split=True, scopes=False, checks=False, **cp):
    scope = jax.named_scope if scopes else (lambda n: contextlib.nullcontext())
    NS = lead + 1
    NA, NB, NC, ND = 8, 32, 8, 8
    GB, GC, GD = NA, NA + NB, NA + NB + NC
    NG = GD + ND
    CR = B * SK // NB
    cs0 = min(cstreams, 32)
    CS = SK // cs0

    def kernel(x_hbm, c_hbm, wq_hbm, wk_hbm, wv_hbm, wo_hbm, w1_hbm, b1_hbm, w2_hbm, b2_hbm, o_ref,
               x_buf, b1_buf, b2_buf, c_buf, wq_buf, wk_buf, wv_buf, wo_buf, w1_buf, w2_buf,
               zt, rows, t8, qa_ref, sc_ref, acc_ref, m_ref, l_ref, ctx8, h_ref,
               sems, sem_small):
        def sem(g):
            return sems.at[g % NS]

        def start(src, dst, g, prio):
            pltpu.make_async_copy(src, dst, sem(g)).start(priority=prio)

        def ds(o, n):
            return pl.ds(o if isinstance(o, int) else pl.multiple_of(o, n), n)

        def issue_a(j, p1=0):
            def rnd(r, prio):
                o = j * 16 + r * 4
                k = 0
                for hbm, buf in ((wq_hbm, wq_buf), (wk_hbm, wk_buf)):
                    for s in range(4):
                        start(hbm.at[s, pl.ds(o, 4)], buf.at[s, pl.ds(o, 4)], j, prio(k))
                        k += 1
            n1 = p1 // 8
            if n1:
                lax.fori_loop(0, n1, lambda r, _: rnd(r, lambda k: 1), None)
            if n1 < 4:
                lax.fori_loop(n1, 4, lambda r, _: rnd(r, lambda k: k % 2), None)

        def issue_b(j):
            b, jj = j // (NB // B), j % (NB // B)
            rounds = CR // 32 // cs0

            def rnd(r, _):
                for s in range(cs0):
                    src = b * SK + s * CS + (jj * rounds + r) * 32
                    dst = (r * cs0 + s) * 32
                    start(c_hbm.at[ds(src, 32)], c_buf.at[j, ds(dst, 32)], GB + j, s % 2)
            lax.fori_loop(0, rounds, rnd, None)

        def issue_c(j):
            def rnd(r, _):
                o, o1 = j * 16 + r * 4, j * 32 + r * 8
                k = 0
                for s in range(4):
                    start(wv_hbm.at[s, pl.ds(o, 4)], wv_buf.at[s, pl.ds(o, 4)], GC + j, k % 2)
                    k += 1
                    if s % 2 == 0:
                        start(w1_hbm.at[s // 2, ds(o1, 8)], w1_buf.at[s // 2, ds(o1, 8)], GC + j, k % 2)
                        k += 1
            lax.fori_loop(0, 4, rnd, None)

        def issue_d(j):
            def rnd(r, _):
                o = j * 128 + r * 32
                k = 0
                for s in range(4):
                    start(wo_hbm.at[s, ds(o, 32)], wo_buf.at[s, ds(o, 32)], GD + j, k % 2)
                    k += 1
                    if s % 2 == 0:
                        start(w2_hbm.at[s // 2, ds(o, 32)], w2_buf.at[s // 2, ds(o, 32)], GD + j, k % 2)
                        k += 1
            lax.fori_loop(0, 4, rnd, None)

        OL = (ND - 1) * 128

        def issue_last():
            k = 0
            for r in range(4):
                for s in range(3 if last_split else 4):
                    o = OL + r * 32
                    start(wo_hbm.at[s, ds(o, 32)], wo_buf.at[s, ds(o, 32)], NG - 1, k % 2)
                    k += 1
            if last_split:
                for r in range(4):
                    o = OL + r * 32
                    pltpu.make_async_copy(wo_hbm.at[3, ds(o, 32)], wo_buf.at[3, ds(o, 32)],
                                          sem_small.at[0]).start(priority=1)

        def wait_ref(ref, g):
            pltpu.make_async_copy(ref, ref, sem(g)).wait()

        def wait_a(j):
            wait_ref(wq_buf.at[:, pl.ds(j * 16, 16)], j)
            wait_ref(wk_buf.at[:, pl.ds(j * 16, 16)], j)

        def wait_b(j):
            wait_ref(c_buf.at[j], GB + j)

        def wait_c(j):
            wait_ref(wv_buf.at[:, pl.ds(j * 16, 16)], GC + j)
            wait_ref(w1_buf.at[:, ds(j * 32, 32)], GC + j)

        def either(first, f, g):
            pl.when(first)(f)
            pl.when(jnp.logical_not(first))(g)

        issue_a(0, head_p1)
        x_copy = pltpu.make_async_copy(x_hbm, x_buf, sem_small.at[0])
        b1_copy = pltpu.make_async_copy(b1_hbm, b1_buf, sem_small.at[1])
        b2_copy = pltpu.make_async_copy(b2_hbm, b2_buf, sem_small.at[1])
        x_copy.start()
        b1_copy.start()
        b2_copy.start()
        lax.fori_loop(1, lead, lambda g, _: issue_a(g), None)

        x_copy.wait()
        x = x_buf[...].astype(F32)
        xc = x - jnp.mean(x, axis=-1, keepdims=True)
        var = jnp.mean(xc * xc, axis=-1, keepdims=True)
        xn = (xc * lax.rsqrt(var + 1e-5)).astype(BF16)
        xf = xn.astype(F32)
        for b in range(B):
            acc_ref[b * H:(b + 1) * H, :] = jnp.broadcast_to(xf[b:b + 1], (H, M))

        def iota(shape, d):
            return lax.broadcasted_iota(I32, shape, d)

        def coef_rows():
            e_of_lane = iota((H, 128), 1) // H

            def body(b, _):
                for s in range(4):
                    z = acc_ref[ds(b * H, H), s * 128:(s + 1) * 128]
                    zt[s] = jnp.concatenate([z] * 4, axis=0).T
                for s in range(4):
                    r = zt[s, pl.ds(0, H, stride=4), :]
                    for e in range(1, 4):
                        r = jnp.where(e_of_lane == e, zt[s, pl.ds(e, H, stride=4), :], r)
                    rows[s, b] = r
            lax.fori_loop(0, B, body, None)

        def head_contract(w_buf, j, r):
            diag = iota((H, 128), 1) % H == iota((H, 128), 0)
            for s in range(4):
                lhs = jnp.concatenate(
                    [jnp.concatenate([jnp.where(diag, rows[s, b, pl.ds(j * 4 + t, 1), :], 0.0) for b in range(B)],
                                     axis=0) for t in range(4)], axis=1).astype(BF16)
                w = w_buf[s, pl.ds(j * 16, 16)].reshape(16 * H, D)
                r = r + jnp.dot(lhs, w, preferred_element_type=F32)
            return r

        coef_rows()
        ctx8[...] = jnp.zeros(ctx8.shape, F32)

        def q_step(j, r):
            with scope('I'):
                either(j + lead < NA, lambda: issue_a(j + lead), lambda: issue_b(j + lead - GB))
            with scope('W'):
                wait_a(j)
            return head_contract(wq_buf, j, r)

        q = lax.fori_loop(0, NA, q_step, jnp.zeros((B * H, D), F32)).astype(BF16)

        QS = 2

        def qa_step(i, _):
            with scope('I'):
                issue_b(i + lead)
            with scope('W'):
                wait_b(i)
            grp = (iota((8, 128), 1) % H) // 8

            def body(k, _):
                kk = i * (16 // QS) + k
                s, c0 = kk // 4, (kk % 4) * 32
                u = wk_buf[s, pl.ds(c0, 32)].reshape(32 * H, D)
                r = lax.dot_general(q, u, NT, preferred_element_type=F32)
                for b in range(B):
                    vs = []
                    for t in range(8):
                        p = [r[b * H + 8 * g:b * H + 8 * g + 8, t * 128:(t + 1) * 128] for g in range(4)]
                        vs.append(jnp.where(grp == 0, p[0], jnp.where(grp == 1, p[1], jnp.where(grp == 2, p[2], p[3]))))
                    t8[b, ds(kk * 64, 64), :] = jnp.concatenate(vs, axis=0)
            lax.fori_loop(0, 16 // QS, body, None)

        lax.fori_loop(0, QS, qa_step, None)

        def qa_final(b, _):
            sub = iota((H, 128), 1) % 8
            e_of_lane = iota((H, 128), 1) % 4
            for s in range(4):
                r = t8[b, pl.ds(s * 256, H, stride=8), :]
                for u in range(1, 8):
                    r = jnp.where(sub == u, t8[b, pl.ds(s * 256 + u, H, stride=8), :], r)
                for e in range(4):
                    zt[s, pl.ds(e, H, stride=4), :] = r
            for s in range(4):
                z = zt[s].T
                r = z[:H]
                for e in range(1, 4):
                    r = jnp.where(e_of_lane == e, z[e * H:(e + 1) * H], r)
                qa_ref[ds(b * H, H), s * 128:(s + 1) * 128] = (r * (D ** -0.5 * LOG2E)).astype(BF16)
        lax.fori_loop(0, B, qa_final, None)

        m_ref[...] = jnp.full((B * H, 128), -jnp.inf, F32)
        l_ref[...] = jnp.zeros((B * H, 128), F32)
        acc_ref[...] = jnp.zeros((B * H, DC), F32)
        sc_ref[...] = jnp.zeros(sc_ref.shape, F32)

        def heads(j):
            return ds((j // (NB // B)) * H, H)

        def attend(j, _):
            g = j + QS
            with scope('I'):
                either(g + lead < NB, lambda: issue_b(g + lead), lambda: issue_c(g + lead - NB))
            with scope('W'):
                either(g < NB, lambda: wait_b(g), lambda: wait_c(g - NB))
            jn, jp = jnp.minimum(j, NB - 1), jnp.maximum(j - 1, 0)
            sc = sc_ref[...]
            sc_ref[...] = lax.dot_general(qa_ref[heads(jn), :], c_buf[jn], NT, preferred_element_type=F32)
            hr = heads(jp)
            m_prev = m_ref[hr, :]
            m_new = jnp.maximum(m_prev, jnp.max(sc, axis=1, keepdims=True))
            p = jnp.exp2(sc - m_new[:, :1])
            alpha = jnp.exp2(m_prev - m_new)
            l_new = alpha * l_ref[hr, :] + jnp.sum(p, axis=1, keepdims=True)
            pv = jnp.dot(p.astype(BF16), c_buf[jp], preferred_element_type=F32)
            acc_new = acc_ref[hr, :] * alpha[:, :1] + pv

            @pl.when(j > 0)
            def _():
                m_ref[hr, :] = m_new
                l_ref[hr, :] = l_new
                acc_ref[hr, :] = acc_new

        lax.fori_loop(0, NB + 1, attend, None)
        acc_ref[...] = acc_ref[...] / l_ref[...][:, :1]
        coef_rows()

        C0 = QS + 1

        def ctx_step(i, r):
            @pl.when(i >= C0)
            def _():
                with scope('I'):
                    either(i + lead < NC, lambda: issue_c(i + lead), lambda: issue_d(i + lead - NC))
                with scope('W'):
                    wait_c(i)
            return head_contract(wv_buf, i, r)

        ctx = lax.fori_loop(0, NC, ctx_step, jnp.zeros((B * H, D), F32))

        issue_d(lead)
        b1_copy.wait()
        b2_copy.wait()
        for b in range(B):
            ctx8[pl.ds(b, H, stride=8), :] = ctx[b * H:(b + 1) * H]
        xn8 = jnp.concatenate([xn, jnp.zeros((16 - B, M), BF16)], axis=0)
        h = jnp.dot(xn8, w1_buf[...].reshape(M, F), preferred_element_type=F32)[:8]
        h = jax.nn.gelu(h + b1_buf[...].astype(F32).reshape(1, F), approximate=True)
        for i in range(F // 128):
            h_ref[i] = h[:, i * 128:(i + 1) * 128]

        def o_part(hh, s, o):
            return jnp.dot(ctx8[ds(hh * 8, 8), :].astype(BF16), wo_buf[s, ds(o, 128), :],
                           preferred_element_type=F32)

        def out_step(j, carry):
            s_acc, g_acc = carry
            g = GD + j

            @pl.when((j > 0) & (g + lead < NG - 1))
            def _():
                issue_d(j + lead)
            pl.when((j > 0) & (g + lead == NG - 1))(issue_last)
            with scope('WD'):
                wait_ref(wo_buf.at[:, ds(j * 128, 128)], g)
                wait_ref(w2_buf.at[:, ds(j * 128, 128)], g)
            for s in range(4):
                s_acc = s_acc + o_part(s * 8 + j, s, j * 128)
            for s in range(2):
                g_acc = g_acc + jnp.dot(h_ref[s * 7 + j].astype(BF16), w2_buf[s, ds(j * 128, 128), :],
                                        preferred_element_type=F32)
            return s_acc, g_acc

        g0 = jnp.broadcast_to(b2_buf[...].astype(F32).reshape(1, M), (8, M))
        s_acc, gg = lax.fori_loop(0, ND - 1, out_step, (jnp.zeros((8, M), F32), g0))
        gate = gg * jax.nn.sigmoid(gg)
        n = 3 if last_split else 4
        with scope('WL'):
            wait_ref(wo_buf.at[pl.ds(0, n), ds(OL, 128)], NG - 1)
        for s in range(n):
            s_acc = s_acc + o_part(s * 8 + ND - 1, s, OL)
        if last_split:
            last = wo_buf.at[3, ds(OL, 128)]
            with scope('WLL'):
                pltpu.make_async_copy(last, last, sem_small.at[0]).wait()
            s_acc = s_acc + o_part(H - 1, 3, OL)
        o_ref[...] = (x + (s_acc * gate)[:B]).astype(BF16)

    if not checks:
        cp = dict(dict(disable_bounds_checks=True, disable_semaphore_checks=True), **cp)

    def fn(A_x, A_c_kv, A_w_q, A_w_uk, A_w_uv, A_w_o, B_x, B_w1, B_b1, B_w2, B_b2):
        out = pl.pallas_call(
            kernel, name=name,
            out_shape=jax.ShapeDtypeStruct((B, M), BF16),
            in_specs=[pl.BlockSpec(memory_space=pltpu.HBM)] * 10,
            out_specs=pl.BlockSpec(memory_space=pltpu.VMEM),
            scratch_shapes=[
                pltpu.VMEM((B, M), BF16), pltpu.VMEM((F,), BF16), pltpu.VMEM((M,), BF16),
                pltpu.VMEM((NB, CR, DC), BF16),
                pltpu.VMEM((4, 128, H, D), BF16), pltpu.VMEM((4, 128, H, D), BF16),
                pltpu.VMEM((4, 128, H, D), BF16), pltpu.VMEM((4, 1024, M), BF16),
                pltpu.VMEM((2, M // 2, F), BF16), pltpu.VMEM((2, F // 2, M), BF16),
                pltpu.VMEM((4, 128, 128), F32), pltpu.VMEM((4, B, H, 128), F32), pltpu.VMEM((B, 1024 + 8, 128), F32),
                pltpu.VMEM((B * H, DC), BF16), pltpu.VMEM((H, CR), F32), pltpu.VMEM((B * H, DC), F32),
                pltpu.VMEM((B * H, 128), F32), pltpu.VMEM((B * H, 128), F32),
                pltpu.VMEM((H * 8 + 8, D), F32), pltpu.VMEM((F // 128, 8, 128), F32),
                pltpu.SemaphoreType.DMA((NS,)), pltpu.SemaphoreType.DMA((2,)),
            ],
            compiler_params=pltpu.CompilerParams(vmem_limit_bytes=100 * 1024 * 1024, **cp),
        )(A_x.reshape(B, M), A_c_kv.reshape(B * SK, DC), A_w_q.reshape(4, 128, H, D),
          A_w_uk.reshape(4, 128, H, D), A_w_uv.reshape(4, 128, H, D), A_w_o.reshape(4, 1024, M),
          B_w1.reshape(2, M // 2, F), B_b1, B_w2.reshape(2, F // 2, M), B_b2)
        return out.reshape(B, 1, M)
    return fn


@jax.jit
def pallas_recurrent_scan__compressed_kv_cla__dense_activation_gelu__decode_kernel(
    A_x, A_c_kv, A_w_q, A_w_uk, A_w_uv, A_w_o, B_x, B_w1, B_b1, B_w2, B_b2,
):
    return make_kernel()(A_x, A_c_kv, A_w_q, A_w_uk, A_w_uv, A_w_o, B_x, B_w1, B_b1, B_w2, B_b2)
```

```python
import jax
import jax.numpy as jnp
from jax import lax
import jax.experimental.pallas as pl
import jax.experimental.pallas.tpu as pltpu

F32 = jnp.float32
BF16 = jnp.bfloat16
I32 = jnp.int32

B, H, SK, D, M, DC, F = 2, 32, 16384, 128, 512, 512, 1792
LOG2E = 1.4426950408889634
NT = (((1,), (1,)), ((), ()))

NA, NB, NC, ND = 8, 32, 8, 8
GB, GC, GD = NA, NA + NB, NA + NB + NC
CR = SK // NB
LEAD = 4
HEAD = 28
SKEW = 24
C_BITS = (1, 9, 5, 7, 8, 6, 0, 2, 3, 4)
ROUND_A = ((0, 0), (1, 0), (1, 1), (0, 1), (0, 2), (1, 2), (1, 3), (0, 3))
ROUND_C = ((0, 0), (0, 1), (0, 2), (0, 3), (1, 0), (1, 1))
ROUND_D = ((0, 0), (0, 2), (1, 0), (1, 1), (0, 1), (0, 3))
ND_LOOP = 5
N_LAST = 16
N_SEMS = GD + ND - 1 + N_LAST


def _iota(shape, dim):
    return lax.broadcasted_iota(I32, shape, dim)


def _ds(o, n):
    return pl.ds(o if isinstance(o, int) else pl.multiple_of(o, n), n)


def _kernel(x_hbm, c_hbm, wq_hbm, wk_hbm, wv_hbm, wo_hbm, w1_hbm, b1_hbm, w2_hbm, b2_hbm, o_ref,
            x_buf, b1_buf, b2_buf, c_buf, wq_buf, wk_buf, wv_buf, wo_buf, w1_buf, w2_buf,
            zt, rows, t8, qa_ref, acc_ref, m_ref, l_ref, ctx8, ctx_t, h_ref, sems, sem_small):
    def start(src, dst, g, prio):
        pltpu.make_async_copy(src, dst, sems.at[g]).start(priority=prio)

    def wait(filled, g):
        pltpu.make_async_copy(filled, filled, sems.at[g]).wait()

    def round_a(j, r, prio):
        i = pl.ds(j * 16 + r * 4, 4)
        for k, (a, s) in enumerate(ROUND_A):
            hbm, buf = ((wq_hbm, wq_buf), (wk_hbm, wk_buf))[a]
            start(hbm.at[s, i], buf.at[s, i], j, prio(k))

    def issue_a(j):
        lax.fori_loop(0, 4, lambda r, _: round_a(j, r, lambda k: k % 2), None)

    def issue_b(j):
        base = sum(((j >> i) & 1) * (32 << C_BITS[5 + i]) for i in range(5))
        fill = [0] * B
        for k in range(32):
            p = sum(((k >> i) & 1) << C_BITS[i] for i in range(5))
            b = p * 32 // SK
            start(c_hbm.at[_ds(base + p * 32, 32)], c_buf.at[j, b, pl.ds(fill[b], 32)], GB + j, k % 2)
            fill[b] += 32

    def issue_c(j):
        def rnd(r, _):
            for k, (a, s) in enumerate(ROUND_C):
                hbm, buf, i = ((wv_hbm, wv_buf, pl.ds(j * 16 + r * 4, 4)),
                               (w1_hbm, w1_buf, _ds(j * 32 + r * 8, 8)))[a]
                start(hbm.at[s, i], buf.at[s, i], GC + j, k % 2)
        lax.fori_loop(0, 4, rnd, None)

    def round_d(j, r):
        i = _ds(j * 128 + r * 32, 32)
        pairs = ((wo_hbm, wo_buf), (w2_hbm, w2_buf))
        return [(pairs[a][0].at[s, i], pairs[a][1].at[s, i]) for a, s in ROUND_D]

    def issue_d(j):
        def rnd(r, _):
            for k, (src, dst) in enumerate(round_d(j, r)):
                start(src, dst, GD + j, k % 2)
        lax.fori_loop(0, 4, rnd, None)

    def last_piece(n):
        i = pl.ds((ND - 1) * 128 + (n % 4) * 32, 32)
        return wo_hbm.at[n // 4, i], wo_buf.at[n // 4, i]

    def issue_end():
        seq = [c + (GD + j,) for j in range(ND_LOOP, ND - 1) for r in range(4) for c in round_d(j, r)]
        seq += [last_piece(n) + (GD + ND - 1 + n,) for n in range(N_LAST)]
        n = len(seq) - 2 * SKEW
        for k in range(n):
            start(*seq[k], k % 2)
        for k in range(n, n + SKEW):
            start(*seq[k], 0)
            start(*seq[k + SKEW], 1)

    for r in range(4):
        round_a(0, r, lambda k: 0 if r * 8 + k == 1 else 1 if r * 8 + k < HEAD else k % 2)
    x_copy = pltpu.make_async_copy(x_hbm, x_buf, sem_small.at[0])
    b1_copy = pltpu.make_async_copy(b1_hbm, b1_buf, sem_small.at[1])
    b2_copy = pltpu.make_async_copy(b2_hbm, b2_buf, sem_small.at[1])
    x_copy.start()
    b1_copy.start()
    b2_copy.start()
    lax.fori_loop(1, LEAD - 1, lambda j, _: issue_a(j), None)

    x_copy.wait()
    x = x_buf[...].astype(F32)
    xc = x - jnp.mean(x, axis=-1, keepdims=True)
    var = jnp.mean(xc * xc, axis=-1, keepdims=True)
    xn = (xc * lax.rsqrt(var + 1e-5)).astype(BF16)
    xf = xn.astype(F32)
    for b in range(B):
        acc_ref[b * H:(b + 1) * H, :] = jnp.broadcast_to(xf[b:b + 1], (H, M))
    issue_a(LEAD - 1)

    def coef_rows():
        e_of_lane = _iota((H, 128), 1) // H
        for b in range(B):
            for s in range(4):
                z = acc_ref[b * H:(b + 1) * H, s * 128:(s + 1) * 128]
                zt[b * 4 + s, 0:128, :] = jnp.concatenate([z] * 4, axis=0).T
        for b in range(B):
            for s in range(4):
                r = zt[b * 4 + s, pl.ds(0, H, stride=4), :]
                for e in range(1, 4):
                    r = jnp.where(e_of_lane == e, zt[b * 4 + s, pl.ds(e, H, stride=4), :], r)
                rows[s, b] = r

    def head_contract(w_buf, j, r):
        diag = _iota((H, 128), 1) % H == _iota((H, 128), 0)
        for s in range(4):
            lhs = jnp.concatenate(
                [jnp.concatenate([jnp.where(diag, rows[s, b, pl.ds(j * 4 + t, 1), :], 0.0) for b in range(B)],
                                 axis=0) for t in range(4)], axis=1).astype(BF16)
            w = w_buf[s, pl.ds(j * 16, 16)].reshape(16 * H, D)
            r = r + jnp.dot(lhs, w, preferred_element_type=F32)
        return r

    coef_rows()

    def q_step(j, r):
        pl.when(j + LEAD < NA)(lambda: issue_a(j + LEAD))
        pl.when(j + LEAD >= NA)(lambda: issue_b(j + LEAD - NA))
        wait(wq_buf.at[:, pl.ds(j * 16, 16)], j)
        wait(wk_buf.at[:, pl.ds(j * 16, 16)], j)
        return head_contract(wq_buf, j, r)

    q = lax.fori_loop(0, NA, q_step, jnp.zeros((B * H, D), F32)).astype(BF16)

    def qa_step(s, _):
        issue_b(LEAD + s)
        grp = (_iota((8, 128), 1) % H) // 8
        r = lax.dot_general(q, wk_buf[s].reshape(128 * H, D), NT, preferred_element_type=F32)
        for b in range(B):
            picked = []
            for t in range(32):
                p = [r[b * H + 8 * g:b * H + 8 * g + 8, t * 128:(t + 1) * 128] for g in range(4)]
                picked.append(jnp.where(grp == 0, p[0],
                                        jnp.where(grp == 1, p[1], jnp.where(grp == 2, p[2], p[3]))))
            t8[b, _ds(s * 256, 256), :] = jnp.concatenate(picked, axis=0)

    lax.fori_loop(0, 4, qa_step, None)
    issue_b(LEAD + 4)
    sub = _iota((H, 128), 1) % 8
    for b in range(B):
        for s in range(4):
            r = t8[b, pl.ds(s * 256, H, stride=8), :]
            for u in range(1, 8):
                r = jnp.where(sub == u, t8[b, pl.ds(s * 256 + u, H, stride=8), :], r)
            for e in range(4):
                zt[b * 4 + s, pl.ds(e, H, stride=4), :] = r
    e_of_lane = _iota((H, 128), 1) % 4
    for b in range(B):
        for s in range(4):
            z = zt[b * 4 + s, 0:128, :].T
            r = z[:H]
            for e in range(1, 4):
                r = jnp.where(e_of_lane == e, z[e * H:(e + 1) * H], r)
            qa_ref[b * H:(b + 1) * H, s * 128:(s + 1) * 128] = (r * (D ** -0.5 * LOG2E)).astype(BF16)

    m_ref[...] = jnp.full((B * H, 128), -jnp.inf, F32)
    l_ref[...] = jnp.zeros((B * H, 128), F32)
    acc_ref[...] = jnp.zeros((B * H, DC), F32)

    def attend(j, _):
        g = j + LEAD + 5
        pl.when(g < NB)(lambda: issue_b(g))
        pl.when((g >= NB) & (g < NB + NC))(lambda: issue_c(g - NB))
        pl.when(g >= NB + NC)(lambda: issue_d(g - NB - NC))
        wait(c_buf.at[j], GB + j)
        sc = [lax.dot_general(qa_ref[b * H:(b + 1) * H, :], c_buf[j, b], NT, preferred_element_type=F32)
              for b in range(B)]
        for b in range(B):
            hr = slice(b * H, (b + 1) * H)
            m_prev = m_ref[hr, :]
            m_new = jnp.maximum(m_prev, jnp.max(sc[b], axis=1, keepdims=True))
            p = jnp.exp2(sc[b] - m_new[:, :1])
            alpha = jnp.exp2(m_prev - m_new)
            l_ref[hr, :] = alpha * l_ref[hr, :] + jnp.sum(p, axis=1, keepdims=True)
            m_ref[hr, :] = m_new
            pv = jnp.dot(p.astype(BF16), c_buf[j, b], preferred_element_type=F32)
            acc_ref[hr, :] = acc_ref[hr, :] * alpha[:, :1] + pv

    lax.fori_loop(0, NB, attend, None)
    next_d = LEAD + 5 - NC
    issue_d(next_d)
    acc_ref[...] = acc_ref[...] / l_ref[...][:, :1]

    coef_rows()

    def ctx_step(j, r):
        g = next_d + 1 + j // 2
        pl.when((j % 2 == 0) & (g < ND_LOOP))(lambda: issue_d(g))
        wait(wv_buf.at[:, pl.ds(j * 16, 16)], GC + j)
        wait(w1_buf.at[:, _ds(j * 32, 32)], GC + j)
        return head_contract(wv_buf, j, r)

    ctx = lax.fori_loop(0, NC, ctx_step, jnp.zeros((B * H, D), F32))
    issue_end()
    ctx8[...] = jnp.zeros(ctx8.shape, F32)
    for b in range(B):
        ctx8[pl.ds(b, H, stride=8), :] = ctx[b * H:(b + 1) * H]
    for s in range(4):
        for b in range(B):
            row = b * H + s * 8 + ND - 1
            ctx_t[s * B + b] = jnp.broadcast_to(ctx[row:row + 1], (128, D)).T

    b1_copy.wait()
    b2_copy.wait()
    xn16 = jnp.concatenate([xn, jnp.zeros((16 - B, M), BF16)], axis=0)
    h = jnp.dot(xn16, w1_buf[...].reshape(M, F), preferred_element_type=F32)[:8]
    h = jax.nn.gelu(h + b1_buf[...].astype(F32).reshape(1, F), approximate=True)
    for i in range(F // 128):
        h_ref[i] = h[:, i * 128:(i + 1) * 128]

    def out_step(j, carry):
        s_acc, g_acc = carry
        i = _ds(j * 128, 128)
        wait(wo_buf.at[:, i], GD + j)
        wait(w2_buf.at[:, i], GD + j)
        for s in range(2):
            g_acc = g_acc + jnp.dot(h_ref[s * 7 + j].astype(BF16), w2_buf[s, i, :],
                                    preferred_element_type=F32)
        for s in range(4):
            s_acc = s_acc + jnp.dot(ctx8[_ds((s * 8 + j) * 8, 8), :].astype(BF16), wo_buf[s, i, :],
                                    preferred_element_type=F32)
        return s_acc, g_acc

    carry = (jnp.zeros((8, M), F32), jnp.broadcast_to(b2_buf[...].astype(F32).reshape(1, M), (8, M)))
    carry = lax.fori_loop(0, ND_LOOP, out_step, carry)
    for j in range(ND_LOOP, ND - 1):
        carry = out_step(j, carry)

    sub8 = _iota((8, 128), 0)

    def fold(a):
        r = a[:, :128]
        for t in range(1, 4):
            r = jnp.where(sub8 // B == t, pltpu.roll(a[:, t * 128:(t + 1) * 128], B * t, 0), r)
        return r

    gate = fold(carry[1])
    gate = gate * jax.nn.sigmoid(gate)
    base = fold(jnp.concatenate([x, jnp.zeros((8 - B, M), F32)], axis=0)) + fold(carry[0]) * gate

    part = [None] * 8
    for n in range(N_LAST):
        _, piece = last_piece(n)
        wait(piece, GD + ND - 1 + n)
        w = piece[...].astype(F32)
        for b in range(B):
            coef = ctx_t[(n // 4) * B + b, pl.ds((n % 4) * 32, 32), :]
            for t in range(4):
                pr = w[:, t * 128:(t + 1) * 128] * coef
                v = (pr[0:8] + pr[8:16]) + (pr[16:24] + pr[24:32])
                part[B * t + b] = v if n == 0 else part[B * t + b] + v
    for d in (4, 2, 1):
        low = (sub8 & d) == 0
        part = [jnp.where(low, part[u] + pltpu.roll(part[u], 8 - d, 0),
                          part[u + d] + pltpu.roll(part[u + d], d, 0)) for u in range(d)]
    out = (base + gate * part[0]).astype(BF16)
    o_ref[...] = jnp.concatenate([out[B * t:B * (t + 1)] for t in range(4)], axis=1)


@jax.jit
def pallas_recurrent_scan__compressed_kv_cla__dense_activation_gelu__decode_kernel(
    A_x: jax.Array,
    A_c_kv: jax.Array,
    A_w_q: jax.Array,
    A_w_uk: jax.Array,
    A_w_uv: jax.Array,
    A_w_o: jax.Array,
    B_x: jax.Array,
    B_w1: jax.Array,
    B_b1: jax.Array,
    B_w2: jax.Array,
    B_b2: jax.Array,
):
    del B_x
    out = pl.pallas_call(
        _kernel,
        out_shape=jax.ShapeDtypeStruct((B, M), BF16),
        in_specs=[pl.BlockSpec(memory_space=pltpu.HBM)] * 10,
        out_specs=pl.BlockSpec(memory_space=pltpu.VMEM),
        scratch_shapes=[
            pltpu.VMEM((B, M), BF16), pltpu.VMEM((F,), BF16), pltpu.VMEM((M,), BF16),
            pltpu.VMEM((NB, B, CR, DC), BF16),
            pltpu.VMEM((4, 128, H, D), BF16), pltpu.VMEM((4, 128, H, D), BF16),
            pltpu.VMEM((4, 128, H, D), BF16), pltpu.VMEM((4, 8 * D, M), BF16),
            pltpu.VMEM((2, M // 2, F), BF16), pltpu.VMEM((2, F // 2, M), BF16),
            pltpu.VMEM((4 * B, 128 + 8, 128), F32), pltpu.VMEM((4, B, H, 128), F32),
            pltpu.VMEM((B, 1024 + 8, 128), F32),
            pltpu.VMEM((B * H, DC), BF16), pltpu.VMEM((B * H, DC), F32),
            pltpu.VMEM((B * H, 128), F32), pltpu.VMEM((B * H, 128), F32),
            pltpu.VMEM((H * 8 + 8, D), F32), pltpu.VMEM((4 * B, 128, 128), F32),
            pltpu.VMEM((F // 128, 8, 128), F32),
            pltpu.SemaphoreType.DMA((N_SEMS,)), pltpu.SemaphoreType.DMA((2,)),
        ],
        compiler_params=pltpu.CompilerParams(
            vmem_limit_bytes=100 * 1024 * 1024,
            disable_bounds_checks=True,
            disable_semaphore_checks=True,
        ),
    )(A_x.reshape(B, M), A_c_kv.reshape(B * SK, DC), A_w_q.reshape(4, 128, H, D),
      A_w_uk.reshape(4, 128, H, D), A_w_uv.reshape(4, 128, H, D), A_w_o.reshape(4, 8 * D, M),
      B_w1.reshape(2, M // 2, F), B_b1, B_w2.reshape(2, F // 2, M), B_b2)
    return out.reshape(B, 1, M)
```

```python
import jax
import jax.numpy as jnp
from jax import lax
import jax.experimental.pallas as pl
import jax.experimental.pallas.tpu as pltpu

F32 = jnp.float32
BF16 = jnp.bfloat16
I32 = jnp.int32

B, H, SK, D, M, DC, F = 2, 32, 16384, 128, 512, 512, 1792
LOG2E = 1.4426950408889634
NT = (((1,), (1,)), ((), ()))

NA, NB, NC, ND = 8, 32, 8, 8
CR = SK // NB
LEAD = 4
HEAD = 28
SKEW = 24
C_BITS = (1, 9, 5, 7, 8, 6, 0, 2, 3, 4)
ROUND_A = ((0, 0), (1, 0), (1, 1), (0, 1), (0, 2), (1, 2), (1, 3), (0, 3))
ROUND_C = ((0, 0), (0, 1), (0, 2), (0, 3), (1, 0), (1, 1))
ROUND_D = ((0, 0), (0, 2), (1, 0), (1, 1), (0, 1), (0, 3))
ND_LOOP = 5
N_LAST = 16


def _iota(shape, dim):
    return lax.broadcasted_iota(I32, shape, dim)


def _ds(o, n):
    return pl.ds(o if isinstance(o, int) else pl.multiple_of(o, n), n)


def _kernel(x_hbm, c_hbm, wq_hbm, wk_hbm, wv_hbm, wo_hbm, w1_hbm, b1_hbm, w2_hbm, b2_hbm, o_ref,
            x_buf, b1_buf, b2_buf, c_buf, wq_buf, wk_buf, wv_buf, wo_buf, w1_buf, w2_buf,
            zt, rows, t8, qa_ref, acc_ref, m_ref, l_ref, ctx8, ctx_t, h_ref,
            sem_a, sem_b, sem_c, sem_d, sem_last, sem_small):
    def start(src, dst, sem, prio):
        pltpu.make_async_copy(src, dst, sem).start(priority=prio)

    def wait(filled, sem):
        pltpu.make_async_copy(filled, filled, sem).wait()

    def round_a(j, r, prio):
        i = pl.ds(j * 16 + r * 4, 4)
        for k, (a, s) in enumerate(ROUND_A):
            hbm, buf = ((wq_hbm, wq_buf), (wk_hbm, wk_buf))[a]
            start(hbm.at[s, i], buf.at[s, i], sem_a.at[2 * j + a], prio(k))

    def issue_a(j):
        lax.fori_loop(0, 4, lambda r, _: round_a(j, r, lambda k: k % 2), None)

    def issue_b(j):
        base = sum(((j >> i) & 1) * (32 << C_BITS[5 + i]) for i in range(5))
        fill = [0] * B
        for k in range(32):
            p = sum(((k >> i) & 1) << C_BITS[i] for i in range(5))
            b = p * 32 // SK
            start(c_hbm.at[_ds(base + p * 32, 32)], c_buf.at[j, b, pl.ds(fill[b], 32)], sem_b.at[j], k % 2)
            fill[b] += 32

    def issue_c(j):
        def rnd(r, _):
            for k, (a, s) in enumerate(ROUND_C):
                hbm, buf, i = ((wv_hbm, wv_buf, pl.ds(j * 16 + r * 4, 4)),
                               (w1_hbm, w1_buf, _ds(j * 32 + r * 8, 8)))[a]
                start(hbm.at[s, i], buf.at[s, i], sem_c.at[2 * j + a], k % 2)
        lax.fori_loop(0, 4, rnd, None)

    def round_d(j, r):
        i = _ds(j * 128 + r * 32, 32)
        pairs = ((wo_hbm, wo_buf), (w2_hbm, w2_buf))
        return [(pairs[a][0].at[s, i], pairs[a][1].at[s, i], sem_d.at[2 * j + a]) for a, s in ROUND_D]

    def issue_d(j):
        def rnd(r, _):
            for k, copy in enumerate(round_d(j, r)):
                start(*copy, k % 2)
        lax.fori_loop(0, 4, rnd, None)

    def last_piece(n):
        i = pl.ds((ND - 1) * 128 + (n % 4) * 32, 32)
        return wo_hbm.at[n // 4, i], wo_buf.at[n // 4, i], sem_last.at[n]

    def issue_end():
        seq = [c for j in range(ND_LOOP, ND - 1) for r in range(4) for c in round_d(j, r)]
        seq += [last_piece(n) for n in range(N_LAST)]
        n = len(seq) - 2 * SKEW
        for k in range(n):
            start(*seq[k], k % 2)
        for k in range(n, n + SKEW):
            start(*seq[k], 0)
            start(*seq[k + SKEW], 1)

    for r in range(4):
        round_a(0, r, lambda k: 0 if r * 8 + k == 1 else 1 if r * 8 + k < HEAD else k % 2)
    x_copy = pltpu.make_async_copy(x_hbm, x_buf, sem_small.at[0])
    b1_copy = pltpu.make_async_copy(b1_hbm, b1_buf, sem_small.at[1])
    b2_copy = pltpu.make_async_copy(b2_hbm, b2_buf, sem_small.at[2])
    x_copy.start()
    b1_copy.start()
    b2_copy.start()
    lax.fori_loop(1, LEAD - 1, lambda j, _: issue_a(j), None)

    x_copy.wait()
    x = x_buf[...].astype(F32)
    xc = x - jnp.mean(x, axis=-1, keepdims=True)
    var = jnp.mean(xc * xc, axis=-1, keepdims=True)
    xn = (xc * lax.rsqrt(var + 1e-5)).astype(BF16)
    xf = xn.astype(F32)
    for b in range(B):
        acc_ref[b * H:(b + 1) * H, :] = jnp.broadcast_to(xf[b:b + 1], (H, M))
    issue_a(LEAD - 1)

    def coef_rows():
        e_of_lane = _iota((H, 128), 1) // H
        for b in range(B):
            for s in range(4):
                z = acc_ref[b * H:(b + 1) * H, s * 128:(s + 1) * 128]
                zt[b * 4 + s, 0:128, :] = jnp.concatenate([z] * 4, axis=0).T
        for b in range(B):
            for s in range(4):
                r = zt[b * 4 + s, pl.ds(0, H, stride=4), :]
                for e in range(1, 4):
                    r = jnp.where(e_of_lane == e, zt[b * 4 + s, pl.ds(e, H, stride=4), :], r)
                rows[s, b] = r

    def head_contract(w_buf, j, r):
        diag = _iota((H, 128), 1) % H == _iota((H, 128), 0)
        for s in range(4):
            lhs = jnp.concatenate(
                [jnp.concatenate([jnp.where(diag, rows[s, b, pl.ds(j * 4 + t, 1), :], 0.0) for b in range(B)],
                                 axis=0) for t in range(4)], axis=1).astype(BF16)
            w = w_buf[s, pl.ds(j * 16, 16)].reshape(16 * H, D)
            r = r + jnp.dot(lhs, w, preferred_element_type=F32)
        return r

    coef_rows()

    def q_step(j, r):
        pl.when(j + LEAD < NA)(lambda: issue_a(j + LEAD))
        pl.when(j + LEAD >= NA)(lambda: issue_b(j + LEAD - NA))
        wait(wq_buf.at[:, pl.ds(j * 16, 16)], sem_a.at[2 * j])
        wait(wk_buf.at[:, pl.ds(j * 16, 16)], sem_a.at[2 * j + 1])
        return head_contract(wq_buf, j, r)

    q = lax.fori_loop(0, NA, q_step, jnp.zeros((B * H, D), F32)).astype(BF16)

    def qa_step(s, _):
        issue_b(LEAD + s)
        grp = (_iota((8, 128), 1) % H) // 8
        r = lax.dot_general(q, wk_buf[s].reshape(128 * H, D), NT, preferred_element_type=F32)
        for b in range(B):
            picked = []
            for t in range(32):
                p = [r[b * H + 8 * g:b * H + 8 * g + 8, t * 128:(t + 1) * 128] for g in range(4)]
                picked.append(jnp.where(grp == 0, p[0],
                                        jnp.where(grp == 1, p[1], jnp.where(grp == 2, p[2], p[3]))))
            t8[b, _ds(s * 256, 256), :] = jnp.concatenate(picked, axis=0)

    lax.fori_loop(0, 4, qa_step, None)
    issue_b(LEAD + 4)
    sub = _iota((H, 128), 1) % 8
    for b in range(B):
        for s in range(4):
            r = t8[b, pl.ds(s * 256, H, stride=8), :]
            for u in range(1, 8):
                r = jnp.where(sub == u, t8[b, pl.ds(s * 256 + u, H, stride=8), :], r)
            for e in range(4):
                zt[b * 4 + s, pl.ds(e, H, stride=4), :] = r
    e_of_lane = _iota((H, 128), 1) % 4
    for b in range(B):
        for s in range(4):
            z = zt[b * 4 + s, 0:128, :].T
            r = z[:H]
            for e in range(1, 4):
                r = jnp.where(e_of_lane == e, z[e * H:(e + 1) * H], r)
            qa_ref[b * H:(b + 1) * H, s * 128:(s + 1) * 128] = (r * (D ** -0.5 * LOG2E)).astype(BF16)

    m_ref[...] = jnp.full((B * H, 128), -jnp.inf, F32)
    l_ref[...] = jnp.zeros((B * H, 128), F32)
    acc_ref[...] = jnp.zeros((B * H, DC), F32)

    def attend(j, _):
        g = j + LEAD + 5
        pl.when(g < NB)(lambda: issue_b(g))
        pl.when((g >= NB) & (g < NB + NC))(lambda: issue_c(g - NB))
        pl.when(g >= NB + NC)(lambda: issue_d(g - NB - NC))
        wait(c_buf.at[j], sem_b.at[j])
        sc = [lax.dot_general(qa_ref[b * H:(b + 1) * H, :], c_buf[j, b], NT, preferred_element_type=F32)
              for b in range(B)]
        for b in range(B):
            hr = slice(b * H, (b + 1) * H)
            m_prev = m_ref[hr, :]
            m_new = jnp.maximum(m_prev, jnp.max(sc[b], axis=1, keepdims=True))
            p = jnp.exp2(sc[b] - m_new[:, :1])
            alpha = jnp.exp2(m_prev - m_new)
            l_ref[hr, :] = alpha * l_ref[hr, :] + jnp.sum(p, axis=1, keepdims=True)
            m_ref[hr, :] = m_new
            pv = jnp.dot(p.astype(BF16), c_buf[j, b], preferred_element_type=F32)
            acc_ref[hr, :] = acc_ref[hr, :] * alpha[:, :1] + pv

    lax.fori_loop(0, NB, attend, None)
    next_d = LEAD + 5 - NC
    issue_d(next_d)
    acc_ref[...] = acc_ref[...] / l_ref[...][:, :1]

    coef_rows()

    def ctx_step(j, r):
        g = next_d + 1 + j // 2
        pl.when((j % 2 == 0) & (g < ND_LOOP))(lambda: issue_d(g))
        wait(wv_buf.at[:, pl.ds(j * 16, 16)], sem_c.at[2 * j])
        wait(w1_buf.at[:, _ds(j * 32, 32)], sem_c.at[2 * j + 1])
        return head_contract(wv_buf, j, r)

    ctx = lax.fori_loop(0, NC, ctx_step, jnp.zeros((B * H, D), F32))
    issue_end()
    ctx8[...] = jnp.zeros(ctx8.shape, F32)
    for b in range(B):
        ctx8[pl.ds(b, H, stride=8), :] = ctx[b * H:(b + 1) * H]
    for s in range(4):
        for b in range(B):
            row = b * H + s * 8 + ND - 1
            ctx_t[s * B + b] = jnp.broadcast_to(ctx[row:row + 1], (128, D)).T

    b1_copy.wait()
    b2_copy.wait()
    xn16 = jnp.concatenate([xn, jnp.zeros((16 - B, M), BF16)], axis=0)
    h = jnp.dot(xn16, w1_buf[...].reshape(M, F), preferred_element_type=F32)[:8]
    h = jax.nn.gelu(h + b1_buf[...].astype(F32).reshape(1, F), approximate=True)
    for i in range(F // 128):
        h_ref[i] = h[:, i * 128:(i + 1) * 128]

    def out_step(j, carry):
        s_acc, g_acc = carry
        i = _ds(j * 128, 128)
        wait(wo_buf.at[:, i], sem_d.at[2 * j])
        wait(w2_buf.at[:, i], sem_d.at[2 * j + 1])
        for s in range(2):
            g_acc = g_acc + jnp.dot(h_ref[s * 7 + j].astype(BF16), w2_buf[s, i, :],
                                    preferred_element_type=F32)
        for s in range(4):
            s_acc = s_acc + jnp.dot(ctx8[_ds((s * 8 + j) * 8, 8), :].astype(BF16), wo_buf[s, i, :],
                                    preferred_element_type=F32)
        return s_acc, g_acc

    carry = (jnp.zeros((8, M), F32), jnp.broadcast_to(b2_buf[...].astype(F32).reshape(1, M), (8, M)))
    carry = lax.fori_loop(0, ND_LOOP, out_step, carry)
    for j in range(ND_LOOP, ND - 1):
        carry = out_step(j, carry)

    sub8 = _iota((8, 128), 0)

    def fold(a):
        r = a[:, :128]
        for t in range(1, 4):
            r = jnp.where(sub8 // B == t, pltpu.roll(a[:, t * 128:(t + 1) * 128], B * t, 0), r)
        return r

    gate = fold(carry[1])
    gate = gate * jax.nn.sigmoid(gate)
    base = fold(jnp.concatenate([x, jnp.zeros((8 - B, M), F32)], axis=0)) + fold(carry[0]) * gate

    part = [None] * 8
    for n in range(N_LAST):
        _, piece, sem = last_piece(n)
        wait(piece, sem)
        w = piece[...].astype(F32)
        for b in range(B):
            coef = ctx_t[(n // 4) * B + b, pl.ds((n % 4) * 32, 32), :]
            for t in range(4):
                pr = w[:, t * 128:(t + 1) * 128] * coef
                v = (pr[0:8] + pr[8:16]) + (pr[16:24] + pr[24:32])
                part[B * t + b] = v if n == 0 else part[B * t + b] + v
    for d in (4, 2, 1):
        low = (sub8 & d) == 0
        part = [jnp.where(low, part[u] + pltpu.roll(part[u], 8 - d, 0),
                          part[u + d] + pltpu.roll(part[u + d], d, 0)) for u in range(d)]
    out = (base + gate * part[0]).astype(BF16)
    o_ref[...] = jnp.concatenate([out[B * t:B * (t + 1)] for t in range(4)], axis=1)


@jax.jit
def pallas_recurrent_scan__compressed_kv_cla__dense_activation_gelu__decode_kernel(
    A_x: jax.Array,
    A_c_kv: jax.Array,
    A_w_q: jax.Array,
    A_w_uk: jax.Array,
    A_w_uv: jax.Array,
    A_w_o: jax.Array,
    B_x: jax.Array,
    B_w1: jax.Array,
    B_b1: jax.Array,
    B_w2: jax.Array,
    B_b2: jax.Array,
):
    del B_x
    out = pl.pallas_call(
        _kernel,
        out_shape=jax.ShapeDtypeStruct((B, M), BF16),
        in_specs=[pl.BlockSpec(memory_space=pltpu.HBM)] * 10,
        out_specs=pl.BlockSpec(memory_space=pltpu.VMEM),
        scratch_shapes=[
            pltpu.VMEM((B, M), BF16), pltpu.VMEM((F,), BF16), pltpu.VMEM((M,), BF16),
            pltpu.VMEM((NB, B, CR, DC), BF16),
            pltpu.VMEM((4, 128, H, D), BF16), pltpu.VMEM((4, 128, H, D), BF16),
            pltpu.VMEM((4, 128, H, D), BF16), pltpu.VMEM((4, 8 * D, M), BF16),
            pltpu.VMEM((2, M // 2, F), BF16), pltpu.VMEM((2, F // 2, M), BF16),
            pltpu.VMEM((4 * B, 128 + 8, 128), F32), pltpu.VMEM((4, B, H, 128), F32),
            pltpu.VMEM((B, 1024 + 8, 128), F32),
            pltpu.VMEM((B * H, DC), BF16), pltpu.VMEM((B * H, DC), F32),
            pltpu.VMEM((B * H, 128), F32), pltpu.VMEM((B * H, 128), F32),
            pltpu.VMEM((H * 8 + 8, D), F32), pltpu.VMEM((4 * B, 128, 128), F32),
            pltpu.VMEM((F // 128, 8, 128), F32),
            pltpu.SemaphoreType.DMA((2 * NA,)), pltpu.SemaphoreType.DMA((NB,)),
            pltpu.SemaphoreType.DMA((2 * NC,)), pltpu.SemaphoreType.DMA((2 * (ND - 1),)),
            pltpu.SemaphoreType.DMA((N_LAST,)), pltpu.SemaphoreType.DMA((3,)),
        ],
        compiler_params=pltpu.CompilerParams(
            vmem_limit_bytes=100 * 1024 * 1024,
            disable_bounds_checks=True,
            disable_semaphore_checks=True,
        ),
    )(A_x.reshape(B, M), A_c_kv.reshape(B * SK, DC), A_w_q.reshape(4, 128, H, D),
      A_w_uk.reshape(4, 128, H, D), A_w_uv.reshape(4, 128, H, D), A_w_o.reshape(4, 8 * D, M),
      B_w1.reshape(2, M // 2, F), B_b1, B_w2.reshape(2, F // 2, M), B_b2)
    return out.reshape(B, 1, M)
```
